```python
import os as _os
_os.environ.setdefault('JAX_PLATFORMS', 'cpu')
import jax
import jax.numpy as jnp

def _softmax(x, axis=-1):
    return jax.nn.softmax(x, axis=axis)

def _gelu(x):
    return jax.nn.gelu(x, approximate=True)

def _silu(x):
    return jax.nn.silu(x)

def _sigmoid(x):
    return jax.nn.sigmoid(x)

def _layernorm(x, axis=-1, eps=1e-05):
    m = jnp.mean(x, axis=axis, keepdims=True)
    v = jnp.var(x, axis=axis, keepdims=True)
    return (x - m) / jnp.sqrt(v + eps)

def _scatter_add(tgt, idx, src, axis=0):
    return tgt.at[idx].add(src)

def _segment_sum(src, seg, n):
    return jax.ops.segment_sum(src, seg, n)

class _Rng:

    def __init__(self, key):
        self._k = key

    def _next(self):
        self._k, sub = jax.random.split(self._k)
        return sub

    def normal(self, shape):
        return jax.random.normal(self._next(), shape, dtype=jnp.bfloat16)

    def randint(self, lo, hi, shape):
        return jax.random.randint(self._next(), shape, lo, hi, dtype=jnp.int32)

    def uniform(self, shape, lo=0.0, hi=1.0):
        return jax.random.uniform(self._next(), shape, jnp.bfloat16, lo, hi)

    def permutation(self, n):
        return jax.random.permutation(self._next(), n)
kernel_name = 'gated_mix__mha_block__memory_aug_recurrent_mem_tr__prompt'

def setup_inputs():
    _rng = _Rng(jax.random.key(int.from_bytes(__import__("os").urandom(4), "little")))
    _w = lambda a: (lambda t: t.astype(jnp.bfloat16) if jnp.issubdtype(t.dtype, jnp.floating) else t)(jnp.asarray(a))

    def _A_setup():
        B, S, D, H = (1, 2048, 512, 32)
        return {'x': _w((lambda *s: _rng.normal(s) * 0.05)(B, S, D)), 'wqkv': _w((lambda *s: _rng.normal(s) * 0.8)(D, 3 * D)), 'wo': _w((lambda *s: _rng.normal(s) * 0.05)(D, D))}
    _A_in = _A_setup()

    def _B_setup():
        B, S, Dm = (1, 2048, 512)
        H, Dh = (32, 128)
        M, seg = (8, 32)
        seg = min(seg, S)
        S = S // seg * seg
        return {'x': _w((lambda *s: _rng.normal(s) * 0.05)(B, S, Dm)), 'mem0': _w((lambda *s: _rng.normal(s) * 0.8)(B, M, Dm)), 'Wq': _w((lambda *s: _rng.normal(s) * 1.6)(Dm, H, Dh) * Dm ** (-0.5)), 'Wk': _w((lambda *s: _rng.normal(s) * 1.6)(Dm, H, Dh) * Dm ** (-0.5)), 'Wv': _w((lambda *s: _rng.normal(s) * 0.8)(Dm, H, Dh) * Dm ** (-0.5)), 'Wo': _w((lambda *s: _rng.normal(s) * 0.8)(H, Dh, Dm) * (H * Dh) ** (-0.5)), 'seg_len': seg}
    _B_in = _B_setup()
    return {'A_x': _A_in['x'], 'A_wqkv': _A_in['wqkv'], 'A_wo': _A_in['wo'], 'B_x': _B_in['x'], 'B_mem0': _B_in['mem0'], 'B_Wq': _B_in['Wq'], 'B_Wk': _B_in['Wk'], 'B_Wv': _B_in['Wv'], 'B_Wo': _B_in['Wo'], 'B_seg_len': _B_in['seg_len'], 'gate_w': _w((lambda *s: _rng.normal(s) * 0.05)(512) * 16.0)}

def reference(A_x, A_wqkv, A_wo, B_x, B_mem0, B_Wq, B_Wk, B_Wv, B_Wo, B_seg_len, gate_w):

    def _A_ref(x, wqkv, wo):
        B, S, D = x.shape
        H = 32
        Dh = D // H
        qkv = (lambda x, *d: x.transpose(*d))((x @ wqkv).reshape(B, S, 3, H, Dh), 2, 0, 3, 1, 4)
        q, k, v = (qkv[0], qkv[1], qkv[2])
        scores = jnp.einsum('bhqd,bhkd->bhqk', q, k) * Dh ** (-0.5)
        p = _softmax(scores, axis=-1)
        o = jnp.einsum('bhqk,bhkd->bhqd', p, v)
        return (lambda x, *d: x.transpose(*d))(o, 0, 2, 1, 3).reshape(B, S, D) @ wo

    def _B_ref(x, mem0, Wq, Wk, Wv, Wo, seg_len):
        B, S, Dm = x.shape
        H, Dh = (Wq.shape[1], Wq.shape[2])
        M = mem0.shape[1]
        scale = Dh ** (-0.5)
        n_seg = S // seg_len
        L = M + seg_len
        idx = jnp.arange(L)
        mask = (idx[:, None] < M) | (idx[:, None] >= idx[None, :])
        mem = mem0
        outs = []
        for s in range(n_seg):
            xs = x[:, s * seg_len:(s + 1) * seg_len, :].copy()
            h = jnp.concatenate([mem, xs], axis=1)
            q = jnp.einsum('btd,dhe->bhte', h, Wq)
            k = jnp.einsum('btd,dhe->bhte', h, Wk)
            v = jnp.einsum('btd,dhe->bhte', h, Wv)
            scores = jnp.einsum('bhqe,bhke->bhqk', q, k) * scale
            scores = jnp.where(mask[None, None], scores, -1000000000.0)
            p = _softmax(scores, axis=-1)
            o = jnp.einsum('bhqk,bhke->bhqe', p, v)
            o = jnp.einsum('bhte,hed->btd', o, Wo)
            mem = o[:, :M, :].copy()
            outs.append(o[:, M:, :])
        return jnp.concatenate(outs, axis=1)
    x = A_x
    g = _sigmoid((x * gate_w).sum(-1, keepdims=True))
    a = _A_ref(x, A_wqkv, A_wo)
    b = _B_ref(x, B_mem0, B_Wq, B_Wk, B_Wv, B_Wo, B_seg_len)
    return g * a + (1 - g) * b
```

```python
import functools

import jax
import jax.numpy as jnp
import jax.experimental.pallas as pl
import jax.experimental.pallas.tpu as pltpu


_LOG2E = 1.4426950408889634

_S = 2048
_D = 512
_HA = 32
_DHA = 16
_HB = 32
_DHB = 128
_M = 8
_SEG = 32
_L = _M + _SEG

_TQ = 512
_CK = 128
_NP = _HB // 2

_F32 = jnp.float32
_BF16 = jnp.bfloat16
_U32 = jnp.uint32


def _b_schedule(lag_v, lag_o):
    seq = [("q", 0), ("k", 0), ("v", 0)]
    done_o = 0
    for t in range(_NP):
        if t + 1 < _NP:
            seq += [("q", t + 1), ("k", t + 1), ("v", t + 1)]
        seq.append(("S", t))
        if t - lag_v >= 0:
            seq.append(("V", t - lag_v))
        if t - lag_o >= 0:
            seq.append(("O", t - lag_o))
            done_o = t - lag_o + 1
    rem_v = list(range(_NP - lag_v, _NP))
    rem_o = list(range(done_o, _NP))
    for i, v in enumerate(rem_v):
        avail = [o for o in rem_o if o < v]
        parts = len(rem_v) - i + 1
        n = -(-len(avail) // parts)
        for o in avail[:n]:
            seq.append(("O", o))
            rem_o.remove(o)
        seq.append(("V", v))
    for o in rem_o:
        seq.append(("O", o))
    return seq


def _recip(l):
    r0 = pl.reciprocal(l, approx=True)
    return r0 * (2.0 - l * r0)


def _kernel(
    x_hbm, wqkv_hbm, woa_hbm, mem0_hbm, wq_hbm, wk_hbm, wv_hbm, wob_hbm, gate_hbm,
    out_hbm,
    x_v, wqkv_v, woa_v, mem0_v, gate_v, stage_v, w2_v, wob_v,
    wt_v, ka_v, qt_v, vt_v, ot_v, sa_v, sb_v, ma_v, mb_v, a_v, out_v,
    sem_in, sem_w, sem_out,
):
    cp_x = pltpu.make_async_copy(x_hbm.at[0], x_v, sem_in.at[0])
    cp_wqkv = pltpu.make_async_copy(wqkv_hbm, wqkv_v, sem_in.at[1])
    cp_woa = pltpu.make_async_copy(woa_hbm, woa_v, sem_in.at[2])
    cp_mem0 = pltpu.make_async_copy(mem0_hbm.at[0], mem0_v, sem_in.at[3])
    cp_gate = pltpu.make_async_copy(gate_hbm, gate_v, sem_in.at[4])
    cp_wqkv.start()
    cp_x.start()
    cp_woa.start()
    cp_mem0.start()
    cp_gate.start()

    w_copies = []
    for mat, w_hbm in enumerate((wq_hbm, wk_hbm, wv_hbm)):
        wu = w_hbm.bitcast(_U32)
        for hp in range(_NP):
            cp = pltpu.make_async_copy(
                wu.at[:, hp, :], stage_v.at[mat * _NP + hp], sem_w.at[mat]
            )
            cp.start()
            w_copies.append(cp)
    for n in range(4):
        cp = pltpu.make_async_copy(
            wob_hbm.at[:, :, pl.ds(n * 128, 128)], wob_v.at[n], sem_w.at[3]
        )
        cp.start()
        w_copies.append(cp)

    cp_wqkv.wait()
    wt_v[pl.ds(0, _D), :] = wqkv_v[:, pl.ds(0, _D)].T
    wt_v[pl.ds(_D, _D), :] = wqkv_v[:, pl.ds(2 * _D, _D)].T
    cp_x.wait()

    a_scale = (_DHA ** -0.5) * _LOG2E
    tb = 256

    def proj_body(i, carry):
        rows = pl.ds(pl.multiple_of(i * tb, tb), tb)
        xb = x_v[rows, :]
        kb = jnp.dot(xb, wqkv_v[:, pl.ds(_D, _D)], preferred_element_type=_F32)
        for g in range(4):
            ka_v[g, rows, :] = kb[:, g * 128:(g + 1) * 128].astype(_BF16)
        qv = jax.lax.dot_general(
            wt_v[...], xb, (((1,), (1,)), ((), ())), preferred_element_type=_F32
        )
        qt_v[:, rows] = (qv[:_D] * a_scale).astype(_BF16)
        vt_v[:, rows] = qv[_D:].astype(_BF16)
        return carry

    jax.lax.fori_loop(0, _S // tb, proj_body, 0)

    nq = _S // _TQ
    nc = _S // _CK
    nu = _HA * nq

    def qpad_of(u):
        h = u // nq
        j = u % nq
        g = h // 8
        qg = qt_v[
            pl.ds(pl.multiple_of(g * 128, 128), 128),
            pl.ds(pl.multiple_of(j * _TQ, _TQ), _TQ),
        ]
        rid = jax.lax.broadcasted_iota(jnp.int32, (128, _TQ), 0) // _DHA
        return g, jnp.where(rid == h % 8, qg, jnp.zeros_like(qg))

    def scores_chunk(g, qpad, c, s_ref, m):
        kc = ka_v[g, pl.ds(c * _CK, _CK), :]
        s = jnp.dot(kc, qpad, preferred_element_type=_F32)
        s_ref[pl.ds(c * _CK, _CK), :] = s
        mc = jnp.max(s.reshape(_CK // 8, 8, _TQ), axis=0)
        return mc if m is None else jnp.maximum(m, mc)

    def pv_chunk(u, c, s_ref, mfin, acc, l8):
        h = u // nq
        p = jnp.exp2(s_ref[pl.ds(c * _CK, _CK), :] - mfin)
        ls = jnp.sum(p.reshape(_CK // 8, 8, _TQ), axis=0)
        vt = vt_v[pl.ds(pl.multiple_of(h * _DHA, _DHA), _DHA), pl.ds(c * _CK, _CK)]
        o = jnp.dot(vt, p.astype(_BF16), preferred_element_type=_F32)
        return (o if acc is None else acc + o), (ls if l8 is None else l8 + ls)

    def finish(u, acc, l8):
        h = u // nq
        j = u % nq
        l = jnp.sum(l8, axis=0, keepdims=True)
        ot_v[
            pl.ds(pl.multiple_of(h * _DHA, _DHA), _DHA),
            pl.ds(pl.multiple_of(j * _TQ, _TQ), _TQ),
        ] = (acc * _recip(l)).astype(_BF16)

    def both(u2, s2_ref, m2_ref, u1, s1_ref, m1_ref):
        mfin = jnp.max(m2_ref[...], axis=0, keepdims=True)
        g, qpad = qpad_of(u1)
        m = acc = l8 = None
        for c in range(nc):
            m = scores_chunk(g, qpad, c, s1_ref, m)
            acc, l8 = pv_chunk(u2, c, s2_ref, mfin, acc, l8)
        m1_ref[...] = m
        finish(u2, acc, l8)

    g0, qpad0 = qpad_of(0)
    m = None
    for c in range(nc):
        m = scores_chunk(g0, qpad0, c, sa_v, m)
    ma_v[...] = m

    def attn_body(i, carry):
        u = 2 * i
        both(u, sa_v, ma_v, u + 1, sb_v, mb_v)
        both(u + 1, sb_v, mb_v, u + 2, sa_v, ma_v)
        return carry

    jax.lax.fori_loop(0, nu // 2 - 1, attn_body, 0)
    both(nu - 2, sa_v, ma_v, nu - 1, sb_v, mb_v)
    mfin = jnp.max(mb_v[...], axis=0, keepdims=True)
    acc = l8 = None
    for c in range(nc):
        acc, l8 = pv_chunk(nu - 1, c, sb_v, mfin, acc, l8)
    finish(nu - 1, acc, l8)

    cp_woa.wait()

    def oproj_body(i, carry):
        cols = pl.ds(pl.multiple_of(i * 512, 512), 512)
        a_v[cols, :] = jax.lax.dot_general(
            ot_v[:, cols], woa_v[...], (((0,), (0,)), ((), ())),
            preferred_element_type=_F32,
        )
        return carry

    jax.lax.fori_loop(0, _S // 512, oproj_body, 0)

    for cp in w_copies:
        cp.wait()

    def repair_body(t, carry):
        mat = t // _NP
        hp = t % _NP
        for blk in range(_D // 16):
            ev = stage_v[t, pl.ds(blk * 16, 8, stride=2), :]
            od = stage_v[t, pl.ds(blk * 16 + 1, 8, stride=2), :]
            w2_v[mat * _HB + 2 * hp, pl.ds(blk * 8, 8), :] = (ev & 0xFFFF) | (od << 16)
            w2_v[mat * _HB + 2 * hp + 1, pl.ds(blk * 8, 8), :] = (
                (ev >> 16) | (od & jnp.uint32(0xFFFF0000))
            )
        return carry

    jax.lax.fori_loop(0, 3 * _NP, repair_body, 0)

    cp_mem0.wait()
    cp_gate.wait()

    b_scale = (_DHB ** -0.5) * _LOG2E
    wobu = wob_v.bitcast(_U32)
    r = jax.lax.broadcasted_iota(jnp.int32, (2 * _L, 2 * _L), 0)
    c_ = jax.lax.broadcasted_iota(jnp.int32, (2 * _L, 2 * _L), 1)
    rh = r >= _L
    ch = c_ >= _L
    ri = jnp.where(rh, r - _L, r)
    ci = jnp.where(ch, c_ - _L, c_)
    mask = (rh == ch) & ((ri < _M) | (ri >= ci))

    def ldw(h):
        return pltpu.bitcast(w2_v[h], _BF16)

    def w_pair(base, p):
        return jnp.concatenate([ldw(base + 2 * p), ldw(base + 2 * p + 1)], axis=1)

    def wo_pair(p):
        return jnp.concatenate(
            [
                jnp.concatenate(
                    [pltpu.bitcast(wobu[n, 2 * p + e], _BF16) for e in range(2)], axis=0
                )
                for n in range(4)
            ],
            axis=1,
        )

    def stack(a):
        return jnp.concatenate([a[:, :_DHB], a[:, _DHB:]], axis=0)

    def step(hb, first, carry_qkv, carry_o):
        st = {}
        acc = None
        new_qkv = {}
        new_o = {}
        for stg, p in _b_schedule(2, 6):
            if stg in ("q", "k", "v"):
                base = {"q": 0, "k": _HB, "v": 2 * _HB}[stg]
                y = jnp.dot(hb, w_pair(base, p), preferred_element_type=_F32)
                if stg == "q":
                    y = y * b_scale
                if first:
                    new_qkv[(stg, p)] = y[_L:_L + 8]
                    y40 = y[:_L]
                else:
                    y40 = jnp.concatenate([y[:_M], carry_qkv[(stg, p)], y[_M:]], axis=0)
                st[(stg, p)] = stack(y40).astype(_BF16)
            elif stg == "S":
                s = jax.lax.dot_general(
                    st.pop(("q", p)), st.pop(("k", p)), (((1,), (1,)), ((), ())),
                    preferred_element_type=_F32,
                )
                s = jnp.where(mask, s, -1e9)
                pe = jnp.exp2(s - jnp.max(s, axis=1, keepdims=True))
                st[("p", p)] = pe.astype(_BF16)
                st[("l", p)] = jnp.sum(pe, axis=1, keepdims=True)
            elif stg == "V":
                o = jnp.dot(st.pop(("p", p)), st.pop(("v", p)), preferred_element_type=_F32)
                o = o * _recip(st.pop(("l", p)))
                o = jnp.concatenate([o[:_L], o[_L:]], axis=1)
                if first:
                    new_o[p] = o[32:_L]
                    st[("o", p)] = o[:32].astype(_BF16)
                else:
                    st[("o", p)] = jnp.concatenate([o, carry_o[p]], axis=0).astype(_BF16)
            else:
                cc = jnp.dot(st.pop(("o", p)), wo_pair(p), preferred_element_type=_F32)
                acc = cc if acc is None else acc + cc
        return acc, new_qkv, new_o

    gate = gate_v[...].reshape(1, _D).astype(_F32)

    def out_copy(i):
        rows = pl.ds(pl.multiple_of(i * 64, 64), 64)
        return pltpu.make_async_copy(out_v.at[rows, :], out_hbm.at[0, rows, :], sem_out.at[0])

    def b_body(i, mem):
        base = pl.multiple_of(i * 64, 64)
        xf = x_v[pl.ds(base, 64), :].astype(_F32)
        h1 = jnp.concatenate([mem, xf[:40]], axis=0).astype(_BF16)
        acc1, cqkv, co = step(h1, True, None, None)
        mem1 = acc1[:_M].astype(_BF16).astype(_F32)
        h2 = jnp.concatenate([mem1, xf[40:64]], axis=0).astype(_BF16)
        acc2, _, _ = step(h2, False, cqkv, co)
        b = jnp.concatenate([acc1[8:32], acc2[40:48], acc2[8:40]], axis=0)
        g = jax.nn.sigmoid(jnp.sum(xf * gate, axis=1, keepdims=True))
        out_v[pl.ds(base, 64), :] = (
            g * a_v[pl.ds(base, 64), :] + (1.0 - g) * b
        ).astype(_BF16)
        out_copy(i).start()
        return acc2[:_M].astype(_BF16).astype(_F32)

    jax.lax.fori_loop(0, _S // 64, b_body, mem0_v[...].astype(_F32))

    def drain(i, carry):
        out_copy(i).wait()
        return carry

    jax.lax.fori_loop(0, _S // 64, drain, 0)


@functools.partial(jax.jit, static_argnames=("B_seg_len",))
def pallas_gated_mix__mha_block__memory_aug_recurrent_mem_tr__prompt_kernel(
    A_x: jax.Array,
    A_wqkv: jax.Array,
    A_wo: jax.Array,
    B_x: jax.Array,
    B_mem0: jax.Array,
    B_Wq: jax.Array,
    B_Wk: jax.Array,
    B_Wv: jax.Array,
    B_Wo: jax.Array,
    B_seg_len: int,
    gate_w: jax.Array,
):
    del B_x
    assert A_x.shape == (1, _S, _D) and B_seg_len == _SEG
    assert B_mem0.shape == (1, _M, _D) and B_Wq.shape == (_D, _HB, _DHB)

    any_spec = pl.BlockSpec(memory_space=pl.ANY)
    scratch = [
        pltpu.VMEM((_S, _D), _BF16),
        pltpu.VMEM((_D, 3 * _D), _BF16),
        pltpu.VMEM((_D, _D), _BF16),
        pltpu.VMEM((_M, _D), _BF16),
        pltpu.VMEM((_D,), _BF16),
        pltpu.VMEM((3 * _NP, _D, _DHB), _U32),
        pltpu.VMEM((3 * _HB, _D // 2, _DHB), _U32),
        pltpu.VMEM((4, _HB, _DHB, 128), _BF16),
        pltpu.VMEM((2 * _D, _D), _BF16),
        pltpu.VMEM((4, _S, 128), _BF16),
        pltpu.VMEM((_D, _S), _BF16),
        pltpu.VMEM((_D, _S), _BF16),
        pltpu.VMEM((_D, _S), _BF16),
        pltpu.VMEM((_S, _TQ), _F32),
        pltpu.VMEM((_S, _TQ), _F32),
        pltpu.VMEM((8, _TQ), _F32),
        pltpu.VMEM((8, _TQ), _F32),
        pltpu.VMEM((_S, _D), _F32),
        pltpu.VMEM((_S, _D), _BF16),
        pltpu.SemaphoreType.DMA((5,)),
        pltpu.SemaphoreType.DMA((4,)),
        pltpu.SemaphoreType.DMA((1,)),
    ]
    return pl.pallas_call(
        _kernel,
        out_shape=jax.ShapeDtypeStruct((1, _S, _D), _BF16),
        in_specs=[any_spec] * 9,
        out_specs=any_spec,
        scratch_shapes=scratch,
        compiler_params=pltpu.CompilerParams(vmem_limit_bytes=100 * 1024 * 1024),
        name="gated_mix",
    )(A_x, A_wqkv, A_wo, B_mem0, B_Wq, B_Wk, B_Wv, B_Wo, gate_w)
```

```python
import functools

import jax
import jax.numpy as jnp
import jax.experimental.pallas as pl
import jax.experimental.pallas.tpu as pltpu


_LOG2E = 1.4426950408889634

_S = 2048
_D = 512
_HA = 32
_DHA = 16
_HB = 32
_DHB = 128
_M = 8
_SEG = 32
_L = _M + _SEG

_TQ = 512
_CK = 128
_TB = 256
_OB = 256
_NP = _HB // 2

_LAG_V = 2
_LAG_O = 6
_BOUNDARY_FILL = 160
_LAST_FILL = 512
_PACE = 2
_RV_EVERY = 3
_PV_PER_BLK = 2
_W_START = [0, 0, 0, 7]
_RMODE = 0

_F32 = jnp.float32
_BF16 = jnp.bfloat16
_U32 = jnp.uint32


def _b_schedule(lag_v, lag_o):
    seq = [("q", 0), ("k", 0), ("v", 0)]
    done_o = 0
    for t in range(_NP):
        if t + 1 < _NP:
            seq += [("q", t + 1), ("k", t + 1), ("v", t + 1)]
        seq.append(("S", t))
        if t - lag_v >= 0:
            seq.append(("V", t - lag_v))
        if t - lag_o >= 0:
            seq.append(("O", t - lag_o))
            done_o = t - lag_o + 1
    rem_v = list(range(_NP - lag_v, _NP))
    rem_o = list(range(done_o, _NP))
    for i, v in enumerate(rem_v):
        avail = [o for o in rem_o if o < v]
        parts = len(rem_v) - i + 1
        for o in avail[: -(-len(avail) // parts)]:
            seq.append(("O", o))
            rem_o.remove(o)
        seq.append(("V", v))
    seq += [("O", o) for o in rem_o]
    return seq


def _merge(main, filler, boundary, boundary_fill):
    tot_m = sum(c for c, _ in main)
    tot_f = sum(c for c, _ in filler)
    out = []
    i_f = 0
    t_f = 0.0
    t_m = 0.0
    for i_m, (c_m, f_m) in enumerate(main):
        target = (t_m / tot_m) * tot_f
        if i_m == boundary:
            target += boundary_fill
        while i_f < len(filler) and t_f + 0.5 * filler[i_f][0] <= target:
            out.append(filler[i_f])
            t_f += filler[i_f][0]
            i_f += 1
        out.append((c_m, f_m))
        t_m += c_m
    return out + filler[i_f:]


def _run(ops):
    for _, thunk in ops:
        thunk()


def _aligned(v, n):
    return v if isinstance(v, int) else pl.multiple_of(v, n)


def _recip(l):
    r0 = pl.reciprocal(l, approx=True)
    return r0 * (2.0 - l * r0)


def _kernel(
    x_hbm, wqkv_hbm, woa_hbm, mem0_hbm, wq_hbm, wk_hbm, wv_hbm, wob_hbm, gate_hbm,
    out_hbm,
    x_v, wqkv_v, woa_v, mem0_v, gate_v, stage_v, w2_v, wob_v,
    wt_v, ka_v, qt_v, vt_v, ot_v, sa_v, sb_v, ma_v, mb_v, b_v, out_v, g_v,
    sem_in, sem_x, sem_w, sem_out,
):
    n_tb = _S // _TB
    nq = _S // _TQ
    nc = _S // _CK
    nu = _HA * nq

    def x_copy(i):
        rows = pl.ds(_aligned(i * _TB, _TB), _TB)
        return pltpu.make_async_copy(x_hbm.at[0, rows, :], x_v.at[rows, :], sem_x.at[i])

    cp_wqkv = pltpu.make_async_copy(wqkv_hbm, wqkv_v, sem_in.at[0])
    cp_woa = pltpu.make_async_copy(woa_hbm, woa_v, sem_in.at[1])
    cp_mem0 = pltpu.make_async_copy(mem0_hbm.at[0], mem0_v, sem_in.at[2])
    cp_gate = pltpu.make_async_copy(gate_hbm, gate_v, sem_in.at[3])

    w_copies = []
    for mat, w_hbm in enumerate((wq_hbm, wk_hbm, wv_hbm)):
        wu = w_hbm.bitcast(_U32)
        w_copies.append([
            pltpu.make_async_copy(wu.at[:, hp, :], stage_v.at[mat * _NP + hp], sem_w.at[mat])
            for hp in range(_NP)
        ])
    w_copies.append([
        pltpu.make_async_copy(wob_hbm.at[:, :, pl.ds(n * 128, 128)], wob_v.at[n], sem_w.at[3])
        for n in range(4)
    ])

    def start_w(mat):
        for cp in w_copies[mat]:
            cp.start()

    def wait_w(mat):
        for cp in w_copies[mat]:
            cp.wait()

    cp_wqkv.start()
    x_copy(0).start()
    cp_gate.start()
    cp_mem0.start()
    cp_wqkv.wait()
    for i in range(1, n_tb):
        x_copy(i).start()
    cp_gate.wait()

    gate = gate_v[...].reshape(1, _D).astype(_F32)
    wt_v[pl.ds(0, _D), :] = wqkv_v[:, pl.ds(0, _D)].T
    wt_v[pl.ds(_D, _D), :] = wqkv_v[:, pl.ds(2 * _D, _D)].T
    a_scale = (_DHA ** -0.5) * _LOG2E

    def repair_unit(t, z=None):
        mat = t // _NP
        hp = t % _NP
        if z is None:
            m_lo, m_hi, s16 = jnp.uint32(0xFFFF), jnp.uint32(0xFFFF0000), jnp.uint32(16)
        else:
            m_lo, m_hi, s16 = z | jnp.uint32(0xFFFF), z | jnp.uint32(0xFFFF0000), z | jnp.uint32(16)
        for blk in range(_D // 16):
            ev = stage_v[t, pl.ds(blk * 16, 8, stride=2), :]
            od = stage_v[t, pl.ds(blk * 16 + 1, 8, stride=2), :]
            w2_v[mat * _HB + 2 * hp, pl.ds(blk * 8, 8), :] = (ev & m_lo) | (od << s16)
            w2_v[mat * _HB + 2 * hp + 1, pl.ds(blk * 8, 8), :] = (ev >> s16) | (od & m_hi)

    def proj_block(i, n_repair):
        for mat in range(4):
            @pl.when(i == _W_START[mat])
            def _():
                start_w(mat)
                if mat == 3:
                    cp_woa.start()

        if n_repair:
            half = n_tb // 2
            for mat in range(2):
                @pl.when(i == half + mat * (half // 2))
                def _():
                    wait_w(mat)

        x_copy(i).wait()
        rows = pl.ds(_aligned(i * _TB, _TB), _TB)
        xb = x_v[rows, :]
        kb = jnp.dot(xb, wqkv_v[:, pl.ds(_D, _D)], preferred_element_type=_F32)
        for g in range(4):
            ka_v[g, rows, :] = kb[:, g * 128:(g + 1) * 128].astype(_BF16)
        qv = jax.lax.dot_general(
            wt_v[...], xb, (((1,), (1,)), ((), ())), preferred_element_type=_F32
        )
        qt_v[:, rows] = (qv[:_D] * a_scale).astype(_BF16)
        vt_v[:, rows] = qv[_D:].astype(_BF16)
        gsum = jnp.sum(xb.astype(_F32) * gate, axis=1, keepdims=True)
        g_v[rows, :] = jnp.broadcast_to(jax.nn.sigmoid(gsum), (_TB, 128))
        for r in range(n_repair):
            repair_unit((i - n_tb // 2) * n_repair + r)

    def first_half(i, c):
        proj_block(i, 0)
        return c

    def second_half(i, c):
        proj_block(i, 2 * _NP // (n_tb // 2))
        return c

    if _RMODE == 1:
        jax.lax.fori_loop(0, n_tb // 2, first_half, 0)
        jax.lax.fori_loop(n_tb // 2, n_tb, second_half, 0)
    else:
        jax.lax.fori_loop(0, n_tb, first_half, 0)

    def qpad_of(u):
        h = u // nq
        j = u % nq
        g = h // 8
        qg = qt_v[pl.ds(_aligned(g * 128, 128), 128), pl.ds(_aligned(j * _TQ, _TQ), _TQ)]
        rid = jax.lax.broadcasted_iota(jnp.int32, (128, _TQ), 0) // _DHA
        return g, jnp.where(rid == h % 8, qg, jnp.zeros_like(qg))

    def scores_chunk(g, qpad, c, s_ref, m):
        s = jnp.dot(ka_v[g, pl.ds(c * _CK, _CK), :], qpad, preferred_element_type=_F32)
        s_ref[pl.ds(c * _CK, _CK), :] = s
        mc = jnp.max(s.reshape(_CK // 8, 8, _TQ), axis=0)
        return mc if m is None else jnp.maximum(m, mc)

    def pv_chunk(u, c, s_ref, m8, acc, l8):
        h = u // nq
        s = s_ref[pl.ds(c * _CK, _CK), :].reshape(_CK // 8, 8, _TQ)
        p = jnp.exp2(s - m8[None])
        ls = jnp.sum(p, axis=0)
        vt = vt_v[pl.ds(_aligned(h * _DHA, _DHA), _DHA), pl.ds(c * _CK, _CK)]
        o = jnp.dot(vt, p.reshape(_CK, _TQ).astype(_BF16), preferred_element_type=_F32)
        return (o if acc is None else acc + o), (ls if l8 is None else l8 + ls)

    def finish(u, acc, l8):
        h = u // nq
        j = u % nq
        l = jnp.sum(l8, axis=0, keepdims=True)
        ot_v[pl.ds(_aligned(h * _DHA, _DHA), _DHA), pl.ds(_aligned(j * _TQ, _TQ), _TQ)] = (
            acc * _recip(l)
        ).astype(_BF16)

    def a_ops(u2, s2_ref, m2_ref, u1, s1_ref, m1_ref, on_pv=None):
        st = {"m": None, "acc": None, "l8": None, "hist": []}
        ops = []

        def prep():
            if u2 is not None:
                mfin = jnp.max(m2_ref[...], axis=0, keepdims=True)
                st["m8"] = jnp.broadcast_to(mfin, (8, _TQ))
            if u1 is not None:
                st["g"], st["qpad"] = qpad_of(u1)

        ops.append((0, prep))
        for c in range(nc):
            def sc(c=c):
                st["m"] = scores_chunk(st["g"], st["qpad"], c, s1_ref, st["m"])

            def pv(c=c):
                m8 = st["m8"]
                if c >= _PACE:
                    m8 = m8 + st["hist"][c - _PACE][:8] * 0.0
                st["acc"], st["l8"] = pv_chunk(u2, c, s2_ref, m8, st["acc"], st["l8"])
                st["hist"].append(st["acc"])
                if on_pv is not None:
                    on_pv(st["acc"])

            if u1 is not None:
                ops.append((_CK, sc))
            if u2 is not None:
                ops.append((32, pv))

        def post():
            if u1 is not None:
                m1_ref[...] = st["m"]
            if u2 is not None:
                finish(u2, st["acc"], st["l8"])

        ops.append((0, post))
        return ops

    _run(a_ops(None, None, None, 0, sa_v, ma_v))
    if _RMODE == 1:
        wait_w(2)
        todo = {"t": 2 * _NP, "n": 0}

        def repair_v(acc):
            todo["n"] += 1
            if todo["n"] % _RV_EVERY == 0 and todo["t"] < 3 * _NP:
                z = pltpu.bitcast(acc[:8, :128] * 0.0, _U32) & jnp.uint32(0x7FFFFFFF)
                repair_unit(todo["t"], z)
                todo["t"] += 1

        _run(a_ops(0, sa_v, ma_v, 1, sb_v, mb_v, repair_v))
        _run(a_ops(1, sb_v, mb_v, 2, sa_v, ma_v, repair_v))
        _run(a_ops(2, sa_v, ma_v, 3, sb_v, mb_v, repair_v))
        while todo["t"] < 3 * _NP:
            repair_unit(todo["t"])
            todo["t"] += 1
    elif _RMODE == 0:
        _run(a_ops(0, sa_v, ma_v, 1, sb_v, mb_v))
        _run(a_ops(1, sb_v, mb_v, 2, sa_v, ma_v))
        _run(a_ops(2, sa_v, ma_v, 3, sb_v, mb_v))
        for mat in range(3):
            wait_w(mat)
        jax.lax.fori_loop(0, 3 * _NP, lambda t, c: (repair_unit(t), c)[1], 0)
    elif _RMODE == 2:
        for mat in range(3):
            wait_w(mat)
        jax.lax.fori_loop(0, 3 * _NP, lambda t, c: (repair_unit(t), c)[1], 0)
        _run(a_ops(0, sa_v, ma_v, 1, sb_v, mb_v))
        _run(a_ops(1, sb_v, mb_v, 2, sa_v, ma_v))
        _run(a_ops(2, sa_v, ma_v, 3, sb_v, mb_v))
    wait_w(3)
    cp_mem0.wait()
    cp_woa.wait()

    b_scale = (_DHB ** -0.5) * _LOG2E
    wobu = wob_v.bitcast(_U32)
    r = jax.lax.broadcasted_iota(jnp.int32, (2 * _L, 2 * _L), 0)
    c_ = jax.lax.broadcasted_iota(jnp.int32, (2 * _L, 2 * _L), 1)
    rh = r >= _L
    ch = c_ >= _L
    ri = jnp.where(rh, r - _L, r)
    ci = jnp.where(ch, c_ - _L, c_)
    mask = (rh == ch) & ((ri < _M) | (ri >= ci))

    def w_pair(base, p):
        return jnp.concatenate(
            [pltpu.bitcast(w2_v[base + 2 * p + e], _BF16) for e in range(2)], axis=1
        )

    def wo_pair(p):
        return jnp.concatenate(
            [
                jnp.concatenate(
                    [pltpu.bitcast(wobu[n, 2 * p + e], _BF16) for e in range(2)], axis=0
                )
                for n in range(4)
            ],
            axis=1,
        )

    def stack(a):
        return jnp.concatenate([a[:, :_DHB], a[:, _DHB:]], axis=0)

    def b_ops(sh, first):
        st = {}
        ops = []
        rows_in = 48 if first else 32
        rows_out = 32 if first else 48

        def begin():
            xs = sh["xf"][:40] if first else sh["xf"][40:64]
            st["hb"] = jnp.concatenate([sh["mem"], xs], axis=0).astype(_BF16)
            st["acc"] = None

        ops.append((0, begin))

        def make(stg, p):
            def proj():
                base = {"q": 0, "k": _HB, "v": 2 * _HB}[stg]
                y = jnp.dot(st["hb"], w_pair(base, p), preferred_element_type=_F32)
                if stg == "q":
                    y = y * b_scale
                if first:
                    sh[("c", stg, p)] = y[_L:_L + 8]
                    y40 = y[:_L]
                else:
                    y40 = jnp.concatenate([y[:_M], sh.pop(("c", stg, p)), y[_M:]], axis=0)
                st[(stg, p)] = stack(y40).astype(_BF16)

            def scores():
                s = jax.lax.dot_general(
                    st.pop(("q", p)), st.pop(("k", p)), (((1,), (1,)), ((), ())),
                    preferred_element_type=_F32,
                )
                s = jnp.where(mask, s, -1e9)
                pe = jnp.exp2(s - jnp.max(s, axis=1, keepdims=True))
                st[("p", p)] = pe.astype(_BF16)
                st[("l", p)] = jnp.sum(pe, axis=1, keepdims=True)

            def values():
                o = jnp.dot(st.pop(("p", p)), st.pop(("v", p)), preferred_element_type=_F32)
                o = o * _recip(st.pop(("l", p)))
                o = jnp.concatenate([o[:_L], o[_L:]], axis=1)
                if first:
                    sh[("co", p)] = o[32:_L]
                    st[("o", p)] = o[:32].astype(_BF16)
                else:
                    st[("o", p)] = jnp.concatenate(
                        [o, sh.pop(("co", p))], axis=0
                    ).astype(_BF16)

            def outproj():
                cc = jnp.dot(st.pop(("o", p)), wo_pair(p), preferred_element_type=_F32)
                st["acc"] = cc if st["acc"] is None else st["acc"] + cc

            if stg in ("q", "k", "v"):
                return (2 * rows_in, proj)
            if stg == "S":
                return (20, scores)
            if stg == "V":
                return (20, values)
            return (2 * rows_out, outproj)

        for stg, p in _b_schedule(_LAG_V, _LAG_O):
            ops.append(make(stg, p))

        def end():
            sh["mem"] = st["acc"][:_M].astype(_BF16).astype(_F32)
            sh["acc1" if first else "acc2"] = st["acc"]

        ops.append((0, end))
        return ops

    def b_trip(base, mem, filler, boundary_fill):
        sh = {"mem": mem, "xf": x_v[pl.ds(base, 64), :].astype(_F32)}
        ops1 = b_ops(sh, True)
        ops2 = b_ops(sh, False)
        _run(_merge(ops1 + ops2, filler, len(ops1), boundary_fill))
        acc1, acc2 = sh["acc1"], sh["acc2"]
        b_v[pl.ds(base, 64), :] = jnp.concatenate(
            [acc1[8:32], acc2[40:48], acc2[8:40]], axis=0
        )
        return sh["mem"]

    def trip(i, mem):
        u = 4 * i + 3
        ops_a = (
            a_ops(u, sb_v, mb_v, u + 1, sa_v, ma_v)
            + a_ops(u + 1, sa_v, ma_v, u + 2, sb_v, mb_v)
            + a_ops(u + 2, sb_v, mb_v, u + 3, sa_v, ma_v)
            + a_ops(u + 3, sa_v, ma_v, u + 4, sb_v, mb_v)
        )
        return b_trip(pl.multiple_of(i * 64, 64), mem, ops_a, _BOUNDARY_FILL)

    mem = jax.lax.fori_loop(0, _S // 64 - 1, trip, mem0_v[...].astype(_F32))

    n_blk = _S // _OB

    def out_copy(blk):
        rows = pl.ds(blk * _OB, _OB)
        return pltpu.make_async_copy(out_v.at[rows, :], out_hbm.at[0, rows, :], sem_out.at[0])

    def a_proj(blk):
        return jax.lax.dot_general(
            ot_v[:, pl.ds(blk * _OB, _OB)], woa_v[...], (((0,), (0,)), ((), ())),
            preferred_element_type=_F32,
        )

    def mix(blk, a):
        rows = pl.ds(blk * _OB, _OB)
        g = g_v[rows, :]
        g = jnp.concatenate([g] * (_D // 128), axis=1)
        out_v[rows, :] = (g * a + (1.0 - g) * b_v[rows, :]).astype(_BF16)
        out_copy(blk).start()

    keep = {}

    def block_op(blk):
        def f():
            a = a_proj(blk)
            if blk < n_blk - 1:
                mix(blk, a)
            else:
                keep["a"] = a

        return (4 * _OB, f)

    last = a_ops(nu - 1, sb_v, mb_v, None, None, None)
    n_free = (nq - 1) * _TQ // _OB
    filler = []
    blk = 0
    while last:
        filler += last[:_PV_PER_BLK]
        last = last[_PV_PER_BLK:]
        if blk < n_free:
            filler.append(block_op(blk))
            blk += 1
    filler += [block_op(b) for b in range(blk, n_blk)]
    b_trip(_S - 64, mem, filler, _LAST_FILL)
    mix(n_blk - 1, keep["a"])
    for b in range(n_blk):
        out_copy(b).wait()


@functools.partial(jax.jit, static_argnames=("B_seg_len",))
def pallas_gated_mix__mha_block__memory_aug_recurrent_mem_tr__prompt_kernel(
    A_x: jax.Array,
    A_wqkv: jax.Array,
    A_wo: jax.Array,
    B_x: jax.Array,
    B_mem0: jax.Array,
    B_Wq: jax.Array,
    B_Wk: jax.Array,
    B_Wv: jax.Array,
    B_Wo: jax.Array,
    B_seg_len: int,
    gate_w: jax.Array,
):
    del B_x
    assert A_x.shape == (1, _S, _D) and B_seg_len == _SEG
    assert B_mem0.shape == (1, _M, _D) and B_Wq.shape == (_D, _HB, _DHB)

    any_spec = pl.BlockSpec(memory_space=pl.ANY)
    scratch = [
        pltpu.VMEM((_S, _D), _BF16),
        pltpu.VMEM((_D, 3 * _D), _BF16),
        pltpu.VMEM((_D, _D), _BF16),
        pltpu.VMEM((_M, _D), _BF16),
        pltpu.VMEM((_D,), _BF16),
        pltpu.VMEM((3 * _NP, _D, _DHB), _U32),
        pltpu.VMEM((3 * _HB, _D // 2, _DHB), _U32),
        pltpu.VMEM((4, _HB, _DHB, 128), _BF16),
        pltpu.VMEM((2 * _D, _D), _BF16),
        pltpu.VMEM((4, _S, 128), _BF16),
        pltpu.VMEM((_D, _S), _BF16),
        pltpu.VMEM((_D, _S), _BF16),
        pltpu.VMEM((_D, _S), _BF16),
        pltpu.VMEM((_S, _TQ), _F32),
        pltpu.VMEM((_S, _TQ), _F32),
        pltpu.VMEM((8, _TQ), _F32),
        pltpu.VMEM((8, _TQ), _F32),
        pltpu.VMEM((_S, _D), _F32),
        pltpu.VMEM((_S, _D), _BF16),
        pltpu.VMEM((_S, 128), _F32),
        pltpu.SemaphoreType.DMA((4,)),
        pltpu.SemaphoreType.DMA((_S // _TB,)),
        pltpu.SemaphoreType.DMA((4,)),
        pltpu.SemaphoreType.DMA((1,)),
    ]
    return pl.pallas_call(
        _kernel,
        out_shape=jax.ShapeDtypeStruct((1, _S, _D), _BF16),
        in_specs=[any_spec] * 9,
        out_specs=any_spec,
        scratch_shapes=scratch,
        compiler_params=pltpu.CompilerParams(vmem_limit_bytes=100 * 1024 * 1024),
        name="gated_mix",
    )(A_x, A_wqkv, A_wo, B_mem0, B_Wq, B_Wk, B_Wv, B_Wo, gate_w)
```

```python
import functools

import jax
import jax.numpy as jnp
import jax.experimental.pallas as pl
import jax.experimental.pallas.tpu as pltpu


_LOG2E = 1.4426950408889634

_S = 2048
_D = 512
_HA = 32
_DHA = 16
_HB = 32
_DHB = 128
_M = 8
_SEG = 32
_L = _M + _SEG

_TQ = 512
_CK = 128
_TB = 256
_OB = 256
_NP = _HB // 2

_LAG_V = 2
_LAG_O = 6
_BOUNDARY_FILL = 160
_LAST_FILL = 512
_PACE = 2
_PACE_LAST = 3
_W_START = (0, 2, 4, 7)

_F32 = jnp.float32
_BF16 = jnp.bfloat16
_U32 = jnp.uint32


def _b_schedule():
    seq = [("q", 0), ("k", 0), ("v", 0)]
    done_o = 0
    for t in range(_NP):
        if t + 1 < _NP:
            seq += [("q", t + 1), ("k", t + 1), ("v", t + 1)]
        seq.append(("S", t))
        if t - _LAG_V >= 0:
            seq.append(("V", t - _LAG_V))
        if t - _LAG_O >= 0:
            seq.append(("O", t - _LAG_O))
            done_o = t - _LAG_O + 1
    rem_v = list(range(_NP - _LAG_V, _NP))
    rem_o = list(range(done_o, _NP))
    for i, v in enumerate(rem_v):
        avail = [o for o in rem_o if o < v]
        parts = len(rem_v) - i + 1
        for o in avail[: -(-len(avail) // parts)]:
            seq.append(("O", o))
            rem_o.remove(o)
        seq.append(("V", v))
    seq += [("O", o) for o in rem_o]
    return seq


def _merge(main, filler, boundary, boundary_fill):
    tot_m = sum(c for c, _ in main)
    tot_f = sum(c for c, _ in filler)
    out = []
    i_f = 0
    t_f = 0.0
    t_m = 0.0
    for i_m, (c_m, f_m) in enumerate(main):
        target = (t_m / tot_m) * tot_f
        if i_m == boundary:
            target += boundary_fill
        while i_f < len(filler) and t_f + 0.5 * filler[i_f][0] <= target:
            out.append(filler[i_f])
            t_f += filler[i_f][0]
            i_f += 1
        out.append((c_m, f_m))
        t_m += c_m
    return out + filler[i_f:]


def _run(ops):
    for _, thunk in ops:
        thunk()


def _aligned(v, n):
    return v if isinstance(v, int) else pl.multiple_of(v, n)


def _recip(l):
    r0 = pl.reciprocal(l, approx=True)
    return r0 * (2.0 - l * r0)


def _kernel(
    x_hbm, wqkv_hbm, woa_hbm, mem0_hbm, wq_hbm, wk_hbm, wv_hbm, wob_hbm, gate_hbm,
    out_hbm,
    x_v, wqkv_v, woa_v, mem0_v, gate_v, stage_v, w2_v, wob_v,
    wt_v, ka_v, qt_v, vt_v, ot_v, sa_v, sb_v, ma_v, mb_v, b_v, out_v, g_v, zero_v,
    sem_in, sem_x, sem_w, sem_out,
):
    n_tb = _S // _TB
    nq = _S // _TQ
    nc = _S // _CK
    nu = _HA * nq

    def x_copy(i):
        rows = pl.ds(_aligned(i * _TB, _TB), _TB)
        return pltpu.make_async_copy(x_hbm.at[0, rows, :], x_v.at[rows, :], sem_x.at[i])

    cp_wqkv = pltpu.make_async_copy(wqkv_hbm, wqkv_v, sem_in.at[0])
    cp_woa = pltpu.make_async_copy(woa_hbm, woa_v, sem_in.at[1])
    cp_mem0 = pltpu.make_async_copy(mem0_hbm.at[0], mem0_v, sem_in.at[2])
    cp_gate = pltpu.make_async_copy(gate_hbm, gate_v, sem_in.at[3])

    w_copies = []
    for mat, w_hbm in enumerate((wq_hbm, wk_hbm, wv_hbm)):
        wu = w_hbm.bitcast(_U32)
        w_copies.append([
            pltpu.make_async_copy(wu.at[:, hp, :], stage_v.at[mat * _NP + hp], sem_w.at[mat])
            for hp in range(_NP)
        ])
    w_copies.append([
        pltpu.make_async_copy(wob_hbm.at[:, :, pl.ds(n * 128, 128)], wob_v.at[n], sem_w.at[3])
        for n in range(4)
    ])

    def start_w(mat):
        for cp in w_copies[mat]:
            cp.start()

    def wait_w(mat):
        for cp in w_copies[mat]:
            cp.wait()

    zero_v[...] = jnp.zeros_like(zero_v)
    cp_wqkv.start()
    x_copy(0).start()
    cp_gate.start()
    cp_mem0.start()
    cp_wqkv.wait()
    for i in range(1, n_tb):
        x_copy(i).start()
    cp_gate.wait()

    masks = {}

    def repair(t, blk, dep):
        if dep is not None:
            z = pltpu.bitcast(dep, _U32) & zero_v[...]
            masks["lo"] = z | jnp.uint32(0xFFFF)
            masks["hi"] = z | jnp.uint32(0xFFFF0000)
            masks["sh"] = z | jnp.uint32(16)
        mat = t // _NP
        hp = t % _NP
        ev = stage_v[t, pl.ds(blk * 16, 8, stride=2), :]
        od = stage_v[t, pl.ds(blk * 16 + 1, 8, stride=2), :]
        w2_v[mat * _HB + 2 * hp, pl.ds(blk * 8, 8), :] = (
            (ev & masks["lo"]) | (od << masks["sh"])
        )
        w2_v[mat * _HB + 2 * hp + 1, pl.ds(blk * 8, 8), :] = (
            (ev >> masks["sh"]) | (od & masks["hi"])
        )

    gate = gate_v[...].reshape(1, _D).astype(_F32)
    wt_v[pl.ds(0, _D), :] = wqkv_v[:, pl.ds(0, _D)].T
    wt_v[pl.ds(_D, _D), :] = wqkv_v[:, pl.ds(2 * _D, _D)].T
    a_scale = (_DHA ** -0.5) * _LOG2E
    half = n_tb // 2
    n_rep = 2 * _NP // half

    def proj_block(i, with_repair):
        for mat in range(4):
            @pl.when(i == _W_START[mat])
            def _():
                start_w(mat)
                if mat == 3:
                    cp_woa.start()

        if with_repair:
            for mat in range(2):
                @pl.when(i == half + mat * (half // 2))
                def _():
                    wait_w(mat)

        x_copy(i).wait()
        rows = pl.ds(_aligned(i * _TB, _TB), _TB)
        xb = x_v[rows, :]
        kb = jnp.dot(xb, wqkv_v[:, pl.ds(_D, _D)], preferred_element_type=_F32)
        for g in range(4):
            ka_v[g, rows, :] = kb[:, g * 128:(g + 1) * 128].astype(_BF16)
        qv = jax.lax.dot_general(
            wt_v[...], xb, (((1,), (1,)), ((), ())), preferred_element_type=_F32
        )
        qt_v[:, rows] = (qv[:_D] * a_scale).astype(_BF16)
        vt_v[:, rows] = qv[_D:].astype(_BF16)
        gsum = jnp.sum(xb.astype(_F32) * gate, axis=1, keepdims=True)
        g_v[rows, :] = jnp.broadcast_to(jax.nn.sigmoid(gsum), (_TB, 128))
        if with_repair:
            for r in range(n_rep):
                for blk in range(_D // 16):
                    row = r * 128 + (blk // 4) * 16
                    dep = qv[row:row + 8, :128] if blk % 4 == 0 else None
                    repair((i - half) * n_rep + r, blk, dep)

    def first_half(i, c):
        proj_block(i, False)
        return c

    def second_half(i, c):
        proj_block(i, True)
        return c

    jax.lax.fori_loop(0, half, first_half, 0)
    jax.lax.fori_loop(half, n_tb, second_half, 0)

    def qpad_of(u):
        h = u // nq
        j = u % nq
        g = h // 8
        qg = qt_v[pl.ds(_aligned(g * 128, 128), 128), pl.ds(_aligned(j * _TQ, _TQ), _TQ)]
        rid = jax.lax.broadcasted_iota(jnp.int32, (128, _TQ), 0) // _DHA
        return g, jnp.where(rid == h % 8, qg, jnp.zeros_like(qg))

    def scores_chunk(g, qpad, c, s_ref, m, hook):
        s = jnp.dot(ka_v[g, pl.ds(c * _CK, _CK), :], qpad, preferred_element_type=_F32)
        s_ref[pl.ds(c * _CK, _CK), :] = s
        if hook is not None:
            hook(s)
        mc = jnp.max(s.reshape(_CK // 8, 8, _TQ), axis=0)
        return mc if m is None else jnp.maximum(m, mc)

    def pv_chunk(u, c, s_ref, m8, acc, l8):
        h = u // nq
        s = s_ref[pl.ds(c * _CK, _CK), :].reshape(_CK // 8, 8, _TQ)
        p = jnp.exp2(s - m8[None])
        ls = jnp.sum(p, axis=0)
        vt = vt_v[pl.ds(_aligned(h * _DHA, _DHA), _DHA), pl.ds(c * _CK, _CK)]
        o = jnp.dot(vt, p.reshape(_CK, _TQ).astype(_BF16), preferred_element_type=_F32)
        return (o if acc is None else acc + o), (ls if l8 is None else l8 + ls)

    def finish(u, acc, l8):
        h = u // nq
        j = u % nq
        l = jnp.sum(l8, axis=0, keepdims=True)
        ot_v[pl.ds(_aligned(h * _DHA, _DHA), _DHA), pl.ds(_aligned(j * _TQ, _TQ), _TQ)] = (
            acc * _recip(l)
        ).astype(_BF16)

    def a_ops(u2, s2_ref, m2_ref, u1, s1_ref, m1_ref, pace=_PACE, hook=None):
        st = {"m": None, "acc": None, "l8": None, "hist": []}
        ops = []

        def prep():
            if u2 is not None:
                mfin = jnp.max(m2_ref[...], axis=0, keepdims=True)
                st["m8"] = jnp.broadcast_to(mfin, (8, _TQ))
            if u1 is not None:
                st["g"], st["qpad"] = qpad_of(u1)

        ops.append((0, prep))
        for c in range(nc):
            def sc(c=c):
                st["m"] = scores_chunk(st["g"], st["qpad"], c, s1_ref, st["m"], hook)

            def pv(c=c):
                m8 = st["m8"]
                if c >= pace:
                    m8 = m8 + st["hist"][c - pace][:8] * 0.0
                st["acc"], st["l8"] = pv_chunk(u2, c, s2_ref, m8, st["acc"], st["l8"])
                st["hist"].append(st["acc"])

            if u1 is not None:
                ops.append((_CK, sc))
            if u2 is not None:
                ops.append((32, pv))

        def post():
            if u1 is not None:
                m1_ref[...] = st["m"]
            if u2 is not None:
                finish(u2, st["acc"], st["l8"])

        ops.append((0, post))
        return ops

    _run(a_ops(None, None, None, 0, sa_v, ma_v))
    wait_w(2)
    work = [(t, blk) for t in range(2 * _NP, 3 * _NP) for blk in range(_D // 16)]

    def repair_some(s):
        for k in range(6):
            for n in range(2):
                if work:
                    t, blk = work.pop(0)
                    repair(t, blk, s[k * 24:k * 24 + 8, :128] if n == 0 else None)

    _run(a_ops(0, sa_v, ma_v, 1, sb_v, mb_v, hook=repair_some))
    _run(a_ops(1, sb_v, mb_v, 2, sa_v, ma_v, hook=repair_some))
    _run(a_ops(2, sa_v, ma_v, 3, sb_v, mb_v, hook=repair_some))
    assert not work
    wait_w(3)
    cp_mem0.wait()
    cp_woa.wait()

    b_scale = (_DHB ** -0.5) * _LOG2E
    wobu = wob_v.bitcast(_U32)
    r = jax.lax.broadcasted_iota(jnp.int32, (2 * _L, 2 * _L), 0)
    c_ = jax.lax.broadcasted_iota(jnp.int32, (2 * _L, 2 * _L), 1)
    rh = r >= _L
    ch = c_ >= _L
    ri = jnp.where(rh, r - _L, r)
    ci = jnp.where(ch, c_ - _L, c_)
    mask = (rh == ch) & ((ri < _M) | (ri >= ci))

    def w_pair(base, p):
        return jnp.concatenate(
            [pltpu.bitcast(w2_v[base + 2 * p + e], _BF16) for e in range(2)], axis=1
        )

    def wo_pair(p):
        return jnp.concatenate(
            [
                jnp.concatenate(
                    [pltpu.bitcast(wobu[n, 2 * p + e], _BF16) for e in range(2)], axis=0
                )
                for n in range(4)
            ],
            axis=1,
        )

    def stack(a):
        return jnp.concatenate([a[:, :_DHB], a[:, _DHB:]], axis=0)

    def b_ops(sh, first):
        st = {}
        ops = []
        rows_in = 48 if first else 32
        rows_out = 32 if first else 48

        def begin():
            xs = sh["xf"][:40] if first else sh["xf"][40:64]
            st["hb"] = jnp.concatenate([sh["mem"], xs], axis=0).astype(_BF16)
            st["acc"] = None

        ops.append((0, begin))

        def make(stg, p):
            def proj():
                base = {"q": 0, "k": _HB, "v": 2 * _HB}[stg]
                y = jnp.dot(st["hb"], w_pair(base, p), preferred_element_type=_F32)
                if stg == "q":
                    y = y * b_scale
                if first:
                    sh[("c", stg, p)] = y[_L:_L + 8]
                    y40 = y[:_L]
                else:
                    y40 = jnp.concatenate([y[:_M], sh.pop(("c", stg, p)), y[_M:]], axis=0)
                st[(stg, p)] = stack(y40).astype(_BF16)

            def scores():
                s = jax.lax.dot_general(
                    st.pop(("q", p)), st.pop(("k", p)), (((1,), (1,)), ((), ())),
                    preferred_element_type=_F32,
                )
                s = jnp.where(mask, s, -1e9)
                pe = jnp.exp2(s - jnp.max(s, axis=1, keepdims=True))
                st[("p", p)] = pe.astype(_BF16)
                st[("l", p)] = jnp.sum(pe, axis=1, keepdims=True)

            def values():
                o = jnp.dot(st.pop(("p", p)), st.pop(("v", p)), preferred_element_type=_F32)
                o = o * _recip(st.pop(("l", p)))
                o = jnp.concatenate([o[:_L], o[_L:]], axis=1)
                if first:
                    sh[("co", p)] = o[32:_L]
                    st[("o", p)] = o[:32].astype(_BF16)
                else:
                    st[("o", p)] = jnp.concatenate(
                        [o, sh.pop(("co", p))], axis=0
                    ).astype(_BF16)

            def outproj():
                cc = jnp.dot(st.pop(("o", p)), wo_pair(p), preferred_element_type=_F32)
                st["acc"] = cc if st["acc"] is None else st["acc"] + cc

            if stg in ("q", "k", "v"):
                return (2 * rows_in, proj)
            if stg == "S":
                return (20, scores)
            if stg == "V":
                return (20, values)
            return (2 * rows_out, outproj)

        for stg, p in _b_schedule():
            ops.append(make(stg, p))

        def end():
            sh["mem"] = st["acc"][:_M].astype(_BF16).astype(_F32)
            sh["acc1" if first else "acc2"] = st["acc"]

        ops.append((0, end))
        return ops

    def b_trip(base, mem, filler, boundary_fill):
        sh = {"mem": mem, "xf": x_v[pl.ds(base, 64), :].astype(_F32)}
        ops1 = b_ops(sh, True)
        ops2 = b_ops(sh, False)
        _run(_merge(ops1 + ops2, filler, len(ops1), boundary_fill))
        acc1, acc2 = sh["acc1"], sh["acc2"]
        b_v[pl.ds(base, 64), :] = jnp.concatenate(
            [acc1[8:32], acc2[40:48], acc2[8:40]], axis=0
        )
        return sh["mem"]

    def trip(i, mem):
        u = 4 * i + 3
        ops_a = (
            a_ops(u, sb_v, mb_v, u + 1, sa_v, ma_v)
            + a_ops(u + 1, sa_v, ma_v, u + 2, sb_v, mb_v)
            + a_ops(u + 2, sb_v, mb_v, u + 3, sa_v, ma_v)
            + a_ops(u + 3, sa_v, ma_v, u + 4, sb_v, mb_v)
        )
        return b_trip(pl.multiple_of(i * 64, 64), mem, ops_a, _BOUNDARY_FILL)

    mem = jax.lax.fori_loop(0, _S // 64 - 1, trip, mem0_v[...].astype(_F32))

    n_blk = _S // _OB
    pieces = [(b * _OB, _OB) for b in range(n_blk - 1)]
    pieces += [(_S - _OB, _OB - 64), (_S - 64, 64)]

    def out_copy(piece):
        r0, n = pieces[piece]
        return pltpu.make_async_copy(
            out_v.at[pl.ds(r0, n), :], out_hbm.at[0, pl.ds(r0, n), :], sem_out.at[0]
        )

    def mix(piece, a):
        r0, n = pieces[piece]
        rows = pl.ds(r0, n)
        g = g_v[rows, :]
        g = jnp.concatenate([g] * (_D // 128), axis=1)
        out_v[rows, :] = (g * a + (1.0 - g) * b_v[rows, :]).astype(_BF16)
        out_copy(piece).start()

    keep = {}

    def block_op(blk):
        def f():
            a = jax.lax.dot_general(
                ot_v[:, pl.ds(blk * _OB, _OB)], woa_v[...], (((0,), (0,)), ((), ())),
                preferred_element_type=_F32,
            )
            if blk < n_blk - 1:
                mix(blk, a)
            else:
                mix(blk, a[:_OB - 64])
                keep["a"] = a[_OB - 64:]

        return (4 * _OB, f)

    last = a_ops(nu - 1, sb_v, mb_v, None, None, None, pace=_PACE_LAST)
    n_free = (nq - 1) * _TQ // _OB
    filler = []
    blk = 0
    while last:
        filler += last[:2]
        last = last[2:]
        if blk < n_free:
            filler.append(block_op(blk))
            blk += 1
    filler += [block_op(b) for b in range(blk, n_blk)]
    b_trip(_S - 64, mem, filler, _LAST_FILL)
    mix(n_blk, keep["a"])
    for piece in range(len(pieces)):
        out_copy(piece).wait()


@functools.partial(jax.jit, static_argnames=("B_seg_len",))
def pallas_gated_mix__mha_block__memory_aug_recurrent_mem_tr__prompt_kernel(
    A_x: jax.Array,
    A_wqkv: jax.Array,
    A_wo: jax.Array,
    B_x: jax.Array,
    B_mem0: jax.Array,
    B_Wq: jax.Array,
    B_Wk: jax.Array,
    B_Wv: jax.Array,
    B_Wo: jax.Array,
    B_seg_len: int,
    gate_w: jax.Array,
):
    del B_x
    assert A_x.shape == (1, _S, _D) and B_seg_len == _SEG
    assert B_mem0.shape == (1, _M, _D) and B_Wq.shape == (_D, _HB, _DHB)

    any_spec = pl.BlockSpec(memory_space=pl.ANY)
    scratch = [
        pltpu.VMEM((_S, _D), _BF16),
        pltpu.VMEM((_D, 3 * _D), _BF16),
        pltpu.VMEM((_D, _D), _BF16),
        pltpu.VMEM((_M, _D), _BF16),
        pltpu.VMEM((_D,), _BF16),
        pltpu.VMEM((3 * _NP, _D, _DHB), _U32),
        pltpu.VMEM((3 * _HB, _D // 2, _DHB), _U32),
        pltpu.VMEM((4, _HB, _DHB, 128), _BF16),
        pltpu.VMEM((2 * _D, _D), _BF16),
        pltpu.VMEM((4, _S, 128), _BF16),
        pltpu.VMEM((_D, _S), _BF16),
        pltpu.VMEM((_D, _S), _BF16),
        pltpu.VMEM((_D, _S), _BF16),
        pltpu.VMEM((_S, _TQ), _F32),
        pltpu.VMEM((_S, _TQ), _F32),
        pltpu.VMEM((8, _TQ), _F32),
        pltpu.VMEM((8, _TQ), _F32),
        pltpu.VMEM((_S, _D), _F32),
        pltpu.VMEM((_S, _D), _BF16),
        pltpu.VMEM((_S, 128), _F32),
        pltpu.VMEM((8, 128), _U32),
        pltpu.SemaphoreType.DMA((4,)),
        pltpu.SemaphoreType.DMA((_S // _TB,)),
        pltpu.SemaphoreType.DMA((4,)),
        pltpu.SemaphoreType.DMA((1,)),
    ]
    return pl.pallas_call(
        _kernel,
        out_shape=jax.ShapeDtypeStruct((1, _S, _D), _BF16),
        in_specs=[any_spec] * 9,
        out_specs=any_spec,
        scratch_shapes=scratch,
        compiler_params=pltpu.CompilerParams(vmem_limit_bytes=100 * 1024 * 1024),
        name="gated_mix",
    )(A_x, A_wqkv, A_wo, B_mem0, B_Wq, B_Wk, B_Wv, B_Wo, gate_w)
```

```python
import functools

import jax
import jax.numpy as jnp
import jax.experimental.pallas as pl
import jax.experimental.pallas.tpu as pltpu


_LOG2E = 1.4426950408889634

_S = 2048
_D = 512
_HA = 32
_DHA = 16
_HB = 32
_DHB = 128
_M = 8
_SEG = 32
_L = _M + _SEG

_TQ = 512
_CK = 128
_TB = 256
_OB = 256
_NP = _HB // 2

_LAG_V = 2
_LAG_O = 6
_BOUNDARY_FILL = 160
_LAST_FILL = 512
_PACE = 2
_PACE_LAST = 3
_W_START = (0, 2, 4, 7)

_F32 = jnp.float32
_BF16 = jnp.bfloat16
_U32 = jnp.uint32


def _b_schedule():
    seq = [("q", 0), ("k", 0), ("v", 0)]
    done_o = 0
    for t in range(_NP):
        if t + 1 < _NP:
            seq += [("q", t + 1), ("k", t + 1), ("v", t + 1)]
        seq.append(("S", t))
        if t - _LAG_V >= 0:
            seq.append(("V", t - _LAG_V))
        if t - _LAG_O >= 0:
            seq.append(("O", t - _LAG_O))
            done_o = t - _LAG_O + 1
    rem_v = list(range(_NP - _LAG_V, _NP))
    rem_o = list(range(done_o, _NP))
    for i, v in enumerate(rem_v):
        avail = [o for o in rem_o if o < v]
        parts = len(rem_v) - i + 1
        for o in avail[: -(-len(avail) // parts)]:
            seq.append(("O", o))
            rem_o.remove(o)
        seq.append(("V", v))
    seq += [("O", o) for o in rem_o]
    return seq


def _merge(main, filler, boundary, boundary_fill):
    tot_m = sum(c for c, _ in main)
    tot_f = sum(c for c, _ in filler)
    out = []
    i_f = 0
    t_f = 0.0
    t_m = 0.0
    for i_m, (c_m, f_m) in enumerate(main):
        target = (t_m / tot_m) * tot_f
        if i_m == boundary:
            target += boundary_fill
        while i_f < len(filler) and t_f + 0.5 * filler[i_f][0] <= target:
            out.append(filler[i_f])
            t_f += filler[i_f][0]
            i_f += 1
        out.append((c_m, f_m))
        t_m += c_m
    return out + filler[i_f:]


def _run(ops):
    for _, thunk in ops:
        thunk()


def _aligned(v, n):
    return v if isinstance(v, int) else pl.multiple_of(v, n)


def _recip(l):
    r0 = pl.reciprocal(l, approx=True)
    return r0 * (2.0 - l * r0)


def _kernel(
    x_hbm, wqkv_hbm, woa_hbm, mem0_hbm, wq_hbm, wk_hbm, wv_hbm, wob_hbm, gate_hbm,
    out_hbm,
    x_v, wqkv_v, woa_v, mem0_v, gate_v, stage_v, w2_v, wob_v,
    wt_v, ka_v, qt_v, vt_v, ot_v, sa_v, sb_v, ma_v, mb_v, b_v, out_v, g_v, zero_v,
    sem_in, sem_x, sem_w, sem_out,
):
    n_tb = _S // _TB
    nq = _S // _TQ
    nc = _S // _CK
    nu = _HA * nq

    def x_copy(i):
        rows = pl.ds(_aligned(i * _TB, _TB), _TB)
        return pltpu.make_async_copy(x_hbm.at[0, rows, :], x_v.at[rows, :], sem_x.at[i])

    cp_wqkv = pltpu.make_async_copy(wqkv_hbm, wqkv_v, sem_in.at[0])
    cp_woa = pltpu.make_async_copy(woa_hbm, woa_v, sem_in.at[1])
    cp_mem0 = pltpu.make_async_copy(mem0_hbm.at[0], mem0_v, sem_in.at[2])
    cp_gate = pltpu.make_async_copy(gate_hbm, gate_v, sem_in.at[3])

    w_copies = []
    for mat, w_hbm in enumerate((wq_hbm, wk_hbm, wv_hbm)):
        wu = w_hbm.bitcast(_U32)
        w_copies.append([
            pltpu.make_async_copy(wu.at[:, hp, :], stage_v.at[mat * _NP + hp], sem_w.at[mat])
            for hp in range(_NP)
        ])
    w_copies.append([
        pltpu.make_async_copy(wob_hbm.at[:, :, pl.ds(n * 128, 128)], wob_v.at[n], sem_w.at[3])
        for n in range(4)
    ])

    def start_w(mat):
        for cp in w_copies[mat]:
            cp.start()

    def wait_w(mat):
        for cp in w_copies[mat]:
            cp.wait()

    zero_v[...] = jnp.zeros_like(zero_v)
    cp_wqkv.start()
    x_copy(0).start()
    cp_gate.start()
    cp_mem0.start()
    cp_wqkv.wait()
    for i in range(1, n_tb):
        x_copy(i).start()
    cp_gate.wait()

    masks = {}

    def repair(t, blk, dep):
        if dep is not None:
            z = pltpu.bitcast(dep, _U32) & zero_v[...]
            masks["lo"] = z | jnp.uint32(0xFFFF)
            masks["hi"] = z | jnp.uint32(0xFFFF0000)
            masks["sh"] = z | jnp.uint32(16)
        mat = t // _NP
        hp = t % _NP
        ev = stage_v[t, pl.ds(blk * 16, 8, stride=2), :]
        od = stage_v[t, pl.ds(blk * 16 + 1, 8, stride=2), :]
        w2_v[mat * _HB + 2 * hp, pl.ds(blk * 8, 8), :] = (
            (ev & masks["lo"]) | (od << masks["sh"])
        )
        w2_v[mat * _HB + 2 * hp + 1, pl.ds(blk * 8, 8), :] = (
            (ev >> masks["sh"]) | (od & masks["hi"])
        )

    gate = gate_v[...].reshape(1, _D).astype(_F32)
    wt_v[pl.ds(0, _D), :] = wqkv_v[:, pl.ds(0, _D)].T
    wt_v[pl.ds(_D, _D), :] = wqkv_v[:, pl.ds(2 * _D, _D)].T
    a_scale = (_DHA ** -0.5) * _LOG2E
    half = n_tb // 2
    n_rep = 2 * _NP // half

    def proj_block(i, with_repair):
        for mat in range(4):
            if (_W_START[mat] >= half) == with_repair:
                @pl.when(i == _W_START[mat])
                def _():
                    start_w(mat)
                    if mat == 3:
                        cp_woa.start()

        if with_repair:
            for mat in range(2):
                @pl.when(i == half + mat * (half // 2))
                def _():
                    wait_w(mat)

        x_copy(i).wait()
        rows = pl.ds(_aligned(i * _TB, _TB), _TB)
        xb = x_v[rows, :]
        kb = jnp.dot(xb, wqkv_v[:, pl.ds(_D, _D)], preferred_element_type=_F32)
        for g in range(4):
            ka_v[g, rows, :] = kb[:, g * 128:(g + 1) * 128].astype(_BF16)
        qv = jax.lax.dot_general(
            wt_v[...], xb, (((1,), (1,)), ((), ())), preferred_element_type=_F32
        )
        qt_v[:, rows] = (qv[:_D] * a_scale).astype(_BF16)
        vt_v[:, rows] = qv[_D:].astype(_BF16)
        gsum = jnp.sum(xb.astype(_F32) * gate, axis=1, keepdims=True)
        g_v[rows, :] = jnp.broadcast_to(jax.nn.sigmoid(gsum), (_TB, 128))
        if with_repair:
            for r in range(n_rep):
                for blk in range(_D // 16):
                    row = r * 128 + (blk // 4) * 16
                    dep = qv[row:row + 8, :128] if blk % 4 == 0 else None
                    repair((i - half) * n_rep + r, blk, dep)

    def first_half(i, c):
        proj_block(i, False)
        return c

    def second_half(i, c):
        proj_block(i, True)
        return c

    jax.lax.fori_loop(0, half, first_half, 0)
    jax.lax.fori_loop(half, n_tb, second_half, 0)

    def qpad_of(u):
        h = u // nq
        j = u % nq
        g = h // 8
        qg = qt_v[pl.ds(_aligned(g * 128, 128), 128), pl.ds(_aligned(j * _TQ, _TQ), _TQ)]
        rid = jax.lax.broadcasted_iota(jnp.int32, (128, _TQ), 0) // _DHA
        return g, jnp.where(rid == h % 8, qg, jnp.zeros_like(qg))

    def scores_chunk(g, qpad, c, s_ref, m, hook):
        s = jnp.dot(ka_v[g, pl.ds(c * _CK, _CK), :], qpad, preferred_element_type=_F32)
        s_ref[pl.ds(c * _CK, _CK), :] = s
        if hook is not None:
            hook(s)
        mc = jnp.max(s.reshape(_CK // 8, 8, _TQ), axis=0)
        return mc if m is None else jnp.maximum(m, mc)

    def pv_chunk(u, c, s_ref, m8, acc, l8):
        h = u // nq
        s = s_ref[pl.ds(c * _CK, _CK), :].reshape(_CK // 8, 8, _TQ)
        p = jnp.exp2(s - m8[None])
        ls = jnp.sum(p, axis=0)
        vt = vt_v[pl.ds(_aligned(h * _DHA, _DHA), _DHA), pl.ds(c * _CK, _CK)]
        o = jnp.dot(vt, p.reshape(_CK, _TQ).astype(_BF16), preferred_element_type=_F32)
        return (o if acc is None else acc + o), (ls if l8 is None else l8 + ls)

    def finish(u, acc, l8):
        h = u // nq
        j = u % nq
        l = jnp.sum(l8, axis=0, keepdims=True)
        ot_v[pl.ds(_aligned(h * _DHA, _DHA), _DHA), pl.ds(_aligned(j * _TQ, _TQ), _TQ)] = (
            acc * _recip(l)
        ).astype(_BF16)

    def a_ops(u2, s2_ref, m2_ref, u1, s1_ref, m1_ref, pace=_PACE, hook=None):
        st = {"m": None, "acc": None, "l8": None, "hist": []}
        ops = []

        def prep():
            if u2 is not None:
                mfin = jnp.max(m2_ref[...], axis=0, keepdims=True)
                st["m8"] = jnp.broadcast_to(mfin, (8, _TQ))
            if u1 is not None:
                st["g"], st["qpad"] = qpad_of(u1)

        ops.append((0, prep))
        for c in range(nc):
            def sc(c=c):
                st["m"] = scores_chunk(st["g"], st["qpad"], c, s1_ref, st["m"], hook)

            def pv(c=c):
                m8 = st["m8"]
                if c >= pace:
                    m8 = m8 + st["hist"][c - pace][:8] * 0.0
                st["acc"], st["l8"] = pv_chunk(u2, c, s2_ref, m8, st["acc"], st["l8"])
                st["hist"].append(st["acc"])

            if u1 is not None:
                ops.append((_CK, sc))
            if u2 is not None:
                ops.append((32, pv))

        def post():
            if u1 is not None:
                m1_ref[...] = st["m"]
            if u2 is not None:
                finish(u2, st["acc"], st["l8"])

        ops.append((0, post))
        return ops

    _run(a_ops(None, None, None, 0, sa_v, ma_v))
    wait_w(2)
    work = [(t, blk) for t in range(2 * _NP, 3 * _NP) for blk in range(_D // 16)]

    def repair_some(s):
        for k in range(6):
            for n in range(2):
                if work:
                    t, blk = work.pop(0)
                    repair(t, blk, s[k * 24:k * 24 + 8, :128] if n == 0 else None)

    _run(a_ops(0, sa_v, ma_v, 1, sb_v, mb_v, hook=repair_some))
    _run(a_ops(1, sb_v, mb_v, 2, sa_v, ma_v, hook=repair_some))
    _run(a_ops(2, sa_v, ma_v, 3, sb_v, mb_v, hook=repair_some))
    assert not work
    wait_w(3)
    cp_mem0.wait()
    cp_woa.wait()

    b_scale = (_DHB ** -0.5) * _LOG2E
    wobu = wob_v.bitcast(_U32)
    r = jax.lax.broadcasted_iota(jnp.int32, (2 * _L, 2 * _L), 0)
    c_ = jax.lax.broadcasted_iota(jnp.int32, (2 * _L, 2 * _L), 1)
    rh = r >= _L
    ch = c_ >= _L
    ri = jnp.where(rh, r - _L, r)
    ci = jnp.where(ch, c_ - _L, c_)
    mask = (rh == ch) & ((ri < _M) | (ri >= ci))

    def w_pair(base, p):
        return jnp.concatenate(
            [pltpu.bitcast(w2_v[base + 2 * p + e], _BF16) for e in range(2)], axis=1
        )

    def wo_pair(p):
        return jnp.concatenate(
            [
                jnp.concatenate(
                    [pltpu.bitcast(wobu[n, 2 * p + e], _BF16) for e in range(2)], axis=0
                )
                for n in range(4)
            ],
            axis=1,
        )

    def stack(a):
        return jnp.concatenate([a[:, :_DHB], a[:, _DHB:]], axis=0)

    def b_ops(sh, first):
        st = {}
        ops = []
        rows_in = 48 if first else 32
        rows_out = 32 if first else 48

        def begin():
            xs = sh["xf"][:40] if first else sh["xf"][40:64]
            st["hb"] = jnp.concatenate([sh["mem"], xs], axis=0).astype(_BF16)
            st["acc"] = None

        ops.append((0, begin))

        def make(stg, p):
            def proj():
                base = {"q": 0, "k": _HB, "v": 2 * _HB}[stg]
                y = jnp.dot(st["hb"], w_pair(base, p), preferred_element_type=_F32)
                if stg == "q":
                    y = y * b_scale
                if first:
                    sh[("c", stg, p)] = y[_L:_L + 8]
                    y40 = y[:_L]
                else:
                    y40 = jnp.concatenate([y[:_M], sh.pop(("c", stg, p)), y[_M:]], axis=0)
                st[(stg, p)] = stack(y40).astype(_BF16)

            def scores():
                s = jax.lax.dot_general(
                    st.pop(("q", p)), st.pop(("k", p)), (((1,), (1,)), ((), ())),
                    preferred_element_type=_F32,
                )
                s = jnp.where(mask, s, -1e9)
                pe = jnp.exp2(s - jnp.max(s, axis=1, keepdims=True))
                st[("p", p)] = pe.astype(_BF16)
                st[("l", p)] = jnp.sum(pe, axis=1, keepdims=True)

            def values():
                o = jnp.dot(st.pop(("p", p)), st.pop(("v", p)), preferred_element_type=_F32)
                o = o * _recip(st.pop(("l", p)))
                o = jnp.concatenate([o[:_L], o[_L:]], axis=1)
                if first:
                    sh[("co", p)] = o[32:_L]
                    st[("o", p)] = o[:32].astype(_BF16)
                else:
                    st[("o", p)] = jnp.concatenate(
                        [o, sh.pop(("co", p))], axis=0
                    ).astype(_BF16)

            def outproj():
                cc = jnp.dot(st.pop(("o", p)), wo_pair(p), preferred_element_type=_F32)
                st["acc"] = cc if st["acc"] is None else st["acc"] + cc

            if stg in ("q", "k", "v"):
                return (2 * rows_in, proj)
            if stg == "S":
                return (20, scores)
            if stg == "V":
                return (20, values)
            return (2 * rows_out, outproj)

        for stg, p in _b_schedule():
            ops.append(make(stg, p))

        def end():
            sh["mem"] = st["acc"][:_M].astype(_BF16).astype(_F32)
            sh["acc1" if first else "acc2"] = st["acc"]

        ops.append((0, end))
        return ops

    def b_trip(base, mem, filler, boundary_fill):
        sh = {"mem": mem, "xf": x_v[pl.ds(base, 64), :].astype(_F32)}
        ops1 = b_ops(sh, True)
        ops2 = b_ops(sh, False)
        _run(_merge(ops1 + ops2, filler, len(ops1), boundary_fill))
        acc1, acc2 = sh["acc1"], sh["acc2"]
        b_v[pl.ds(base, 64), :] = jnp.concatenate(
            [acc1[8:32], acc2[40:48], acc2[8:40]], axis=0
        )
        return sh["mem"]

    def trip(i, mem):
        u = 4 * i + 3
        ops_a = (
            a_ops(u, sb_v, mb_v, u + 1, sa_v, ma_v)
            + a_ops(u + 1, sa_v, ma_v, u + 2, sb_v, mb_v)
            + a_ops(u + 2, sb_v, mb_v, u + 3, sa_v, ma_v)
            + a_ops(u + 3, sa_v, ma_v, u + 4, sb_v, mb_v)
        )
        return b_trip(pl.multiple_of(i * 64, 64), mem, ops_a, _BOUNDARY_FILL)

    mem = jax.lax.fori_loop(0, _S // 64 - 1, trip, mem0_v[...].astype(_F32))

    n_blk = _S // _OB
    pieces = [(b * _OB, _OB) for b in range(n_blk - 1)]
    pieces += [(_S - _OB, _OB - 64), (_S - 64, 64)]

    def out_copy(piece):
        r0, n = pieces[piece]
        return pltpu.make_async_copy(
            out_v.at[pl.ds(r0, n), :], out_hbm.at[0, pl.ds(r0, n), :], sem_out.at[0]
        )

    def mix(piece, a):
        r0, n = pieces[piece]
        rows = pl.ds(r0, n)
        g = g_v[rows, :]
        g = jnp.concatenate([g] * (_D // 128), axis=1)
        out_v[rows, :] = (g * a + (1.0 - g) * b_v[rows, :]).astype(_BF16)
        out_copy(piece).start()

    keep = {}

    def block_op(blk):
        def f():
            a = jax.lax.dot_general(
                ot_v[:, pl.ds(blk * _OB, _OB)], woa_v[...], (((0,), (0,)), ((), ())),
                preferred_element_type=_F32,
            )
            if blk < n_blk - 1:
                mix(blk, a)
            else:
                mix(blk, a[:_OB - 64])
                keep["a"] = a[_OB - 64:]

        return (4 * _OB, f)

    last = a_ops(nu - 1, sb_v, mb_v, None, None, None, pace=_PACE_LAST)
    n_free = (nq - 1) * _TQ // _OB
    filler = []
    blk = 0
    while last:
        filler += last[:2]
        last = last[2:]
        if blk < n_free:
            filler.append(block_op(blk))
            blk += 1
    filler += [block_op(b) for b in range(blk, n_blk)]
    b_trip(_S - 64, mem, filler, _LAST_FILL)
    mix(n_blk, keep["a"])
    for piece in range(len(pieces)):
        out_copy(piece).wait()


@functools.partial(jax.jit, static_argnames=("B_seg_len",))
def pallas_gated_mix__mha_block__memory_aug_recurrent_mem_tr__prompt_kernel(
    A_x: jax.Array,
    A_wqkv: jax.Array,
    A_wo: jax.Array,
    B_x: jax.Array,
    B_mem0: jax.Array,
    B_Wq: jax.Array,
    B_Wk: jax.Array,
    B_Wv: jax.Array,
    B_Wo: jax.Array,
    B_seg_len: int,
    gate_w: jax.Array,
):
    del B_x
    assert A_x.shape == (1, _S, _D) and B_seg_len == _SEG
    assert B_mem0.shape == (1, _M, _D) and B_Wq.shape == (_D, _HB, _DHB)

    any_spec = pl.BlockSpec(memory_space=pl.ANY)
    scratch = [
        pltpu.VMEM((_S, _D), _BF16),
        pltpu.VMEM((_D, 3 * _D), _BF16),
        pltpu.VMEM((_D, _D), _BF16),
        pltpu.VMEM((_M, _D), _BF16),
        pltpu.VMEM((_D,), _BF16),
        pltpu.VMEM((3 * _NP, _D, _DHB), _U32),
        pltpu.VMEM((3 * _HB, _D // 2, _DHB), _U32),
        pltpu.VMEM((4, _HB, _DHB, 128), _BF16),
        pltpu.VMEM((2 * _D, _D), _BF16),
        pltpu.VMEM((4, _S, 128), _BF16),
        pltpu.VMEM((_D, _S), _BF16),
        pltpu.VMEM((_D, _S), _BF16),
        pltpu.VMEM((_D, _S), _BF16),
        pltpu.VMEM((_S, _TQ), _F32),
        pltpu.VMEM((_S, _TQ), _F32),
        pltpu.VMEM((8, _TQ), _F32),
        pltpu.VMEM((8, _TQ), _F32),
        pltpu.VMEM((_S, _D), _F32),
        pltpu.VMEM((_S, _D), _BF16),
        pltpu.VMEM((_S, 128), _F32),
        pltpu.VMEM((8, 128), _U32),
        pltpu.SemaphoreType.DMA((4,)),
        pltpu.SemaphoreType.DMA((_S // _TB,)),
        pltpu.SemaphoreType.DMA((4,)),
        pltpu.SemaphoreType.DMA((1,)),
    ]
    return pl.pallas_call(
        _kernel,
        out_shape=jax.ShapeDtypeStruct((1, _S, _D), _BF16),
        in_specs=[any_spec] * 9,
        out_specs=any_spec,
        scratch_shapes=scratch,
        compiler_params=pltpu.CompilerParams(vmem_limit_bytes=100 * 1024 * 1024),
        name="gated_mix",
    )(A_x, A_wqkv, A_wo, B_mem0, B_Wq, B_Wk, B_Wv, B_Wo, gate_w)
```
